```python
import jax
import jax.numpy as jnp

def _softmax(x, axis=-1):
    return jax.nn.softmax(x, axis=axis)
def _gelu(x):
    return jax.nn.gelu(x, approximate=True)
def _silu(x):
    return jax.nn.silu(x)
def _sigmoid(x):
    return jax.nn.sigmoid(x)
def _layernorm(x, axis=-1, eps=1e-5):
    m = jnp.mean(x, axis=axis, keepdims=True)
    v = jnp.var(x, axis=axis, keepdims=True)
    return (x - m) / jnp.sqrt(v + eps)
def _scatter_add(tgt, idx, src, axis=0):
    return tgt.at[idx].add(src)
def _segment_sum(src, seg, n):
    return jax.ops.segment_sum(src, seg, n)
class _Rng:
    def __init__(self, key):
        self._k = key
    def _next(self):
        self._k, sub = jax.random.split(self._k)
        return sub
    def normal(self, shape):
        return jax.random.normal(self._next(), shape, dtype=jnp.bfloat16)
    def randint(self, lo, hi, shape):
        return jax.random.randint(self._next(), shape, lo, hi, dtype=jnp.int32)
    def uniform(self, shape, lo=0.0, hi=1.0):
        return jax.random.uniform(self._next(), shape, jnp.bfloat16, lo, hi)
    def permutation(self, n):
        return jax.random.permutation(self._next(), n)


kernel_name = 'standalone__winograd__vision'

def setup_inputs():
    _rng = _Rng(jax.random.key(int.from_bytes(__import__("os").urandom(4), "little")))
    _w = (lambda a: (lambda t: t.astype(jnp.bfloat16) if jnp.issubdtype(t.dtype, jnp.floating) else t)(jnp.asarray(a)))
    H = W = 512 // 2 * 2
    C = 192
    return {
        "x": _w((lambda *s: _rng.normal(s) * 0.05)(1, H, W, C)),
        "w": _w((lambda *s: _rng.normal(s) * 0.05)(3, 3, C, C)),
    }

def reference(x, w):
    N, H, W, C = x.shape
    K = w.shape[-1]
    G  = jnp.array([[1.0,0.0,0.0],[0.5,0.5,0.5],[0.5,-0.5,0.5],[0.0,0.0,1.0]], dtype=x.dtype)
    Bt = jnp.array([[1.0,0.0,-1.0,0.0],[0.0,1.0,1.0,0.0],[0.0,-1.0,1.0,0.0],[0.0,1.0,0.0,-1.0]], dtype=x.dtype)
    At = jnp.array([[1.0,1.0,1.0,0.0],[0.0,1.0,-1.0,-1.0]], dtype=x.dtype)
    U = jnp.einsum("ar,rsck,bs->abck", G, w, G)
    xp = jnp.pad(x, ((0,0),(1,1),(1,1),(0,0)))
    nH, nW = H // 2, W // 2
    patches = []
    for i in range(4):
        for j in range(4):
            patches.append(xp[:, i:i + 2 * nH:2, j:j + 2 * nW:2, :])
    d = jnp.stack(patches).reshape(4, 4, N * nH * nW, C)
    V = jnp.einsum("ai,ijpc,bj->abpc", Bt, d, Bt)
    M = jnp.einsum("abck,abpc->abpk", U, V)
    Y = jnp.einsum("ma,abpk,nb->pmnk", At, M, At)
    Y = Y.reshape(N, nH, nW, 2, 2, K)
    Y = (lambda x, *d: x.transpose(*d))(Y, 0, 1, 3, 2, 4, 5).reshape(N, H, W, K)
    return Y
```

```python
import jax
import jax.numpy as jnp
import numpy as np
import jax.experimental.pallas as pl
import jax.experimental.pallas.tpu as pltpu

TH = 16
_G = np.array([[1 / 4, 0, 0], [-1 / 6, -1 / 6, -1 / 6], [-1 / 6, 1 / 6, -1 / 6],
               [1 / 24, 1 / 12, 1 / 6], [1 / 24, -1 / 12, 1 / 6], [0, 0, 1]], np.float32)


def _kernel(prev_ref, x_ref, next_ref, w_ref, o_ref, u_ref):
    i = pl.program_id(0)
    C, W = x_ref.shape[1], x_ref.shape[2]

    @pl.when(i == 0)
    def _():
        g = [w_ref[r].astype(jnp.float32) for r in range(3)]
        for a in range(6):
            acc = None
            for r in range(3):
                if _G[a, r] != 0:
                    t = g[r] * float(_G[a, r])
                    acc = t if acc is None else acc + t
            u_ref[a] = acc.astype(jnp.bfloat16)

    def row(j):
        if j < 0:
            return jnp.where(i > 0, prev_ref[0].astype(jnp.float32), 0.0)
        if j >= TH:
            return jnp.where(i < pl.num_programs(0) - 1,
                             next_ref[0].astype(jnp.float32), 0.0)
        return x_ref[j].astype(jnp.float32)

    lane = jax.lax.broadcasted_iota(jnp.int32, (C // 2, W), 1)

    def mm(a, v):
        vb = v.astype(jnp.bfloat16)
        vu = pltpu.bitcast(vb, jnp.uint32)
        zero = jnp.zeros_like(vu)
        l = jnp.where(lane == 0, zero, pltpu.roll(vu, 1, 1))
        r = jnp.where(lane == W - 1, zero, pltpu.roll(vu, W - 1, 1))
        cat = jnp.concatenate(
            [pltpu.bitcast(l, jnp.bfloat16), vb, pltpu.bitcast(r, jnp.bfloat16)], axis=0)
        return jnp.dot(u_ref[a], cat, preferred_element_type=jnp.float32)

    for q in range(TH // 4):
        d0, d1, d2, d3, d4, d5 = [row(4 * q - 1 + k) for k in range(6)]
        p = d4 - 4.0 * d2
        s = d3 - 4.0 * d1
        e = d4 - d2
        f = 2.0 * (d3 - d1)
        m1 = mm(1, p + s)
        m2 = mm(2, p - s)
        m3 = mm(3, e + f)
        m4 = mm(4, e - f)
        s12, d12, s34, d34 = m1 + m2, m1 - m2, m3 + m4, m3 - m4
        m0 = mm(0, 4.0 * (d0 - d2) + e)
        o_ref[4 * q] = (m0 + s12 + s34).astype(o_ref.dtype)
        o_ref[4 * q + 1] = (d12 + 2.0 * d34).astype(o_ref.dtype)
        o_ref[4 * q + 2] = (s12 + 4.0 * s34).astype(o_ref.dtype)
        m5 = mm(5, 4.0 * (d1 - d3) + (d5 - d3))
        o_ref[4 * q + 3] = (d12 + 8.0 * d34 + m5).astype(o_ref.dtype)


@jax.jit
def pallas_standalone__winograd__vision_kernel(x: jax.Array, w: jax.Array):
    N, H, W, C = x.shape
    K = w.shape[-1]
    assert N == 1 and H % TH == 0
    xt = x.reshape(H, W, C).transpose(0, 2, 1)
    wt = w.transpose(0, 3, 1, 2).reshape(3, K, 3 * C)
    out = pl.pallas_call(
        _kernel,
        grid=(H // TH,),
        in_specs=[
            pl.BlockSpec((1, C, W), lambda i: (jnp.maximum(i * TH - 1, 0), 0, 0)),
            pl.BlockSpec((TH, C, W), lambda i: (i, 0, 0)),
            pl.BlockSpec((1, C, W), lambda i: (jnp.minimum(i * TH + TH, H - 1), 0, 0)),
            pl.BlockSpec((3, K, 3 * C), lambda i: (0, 0, 0)),
        ],
        out_specs=pl.BlockSpec((TH, K, W), lambda i: (i, 0, 0)),
        out_shape=jax.ShapeDtypeStruct((H, K, W), x.dtype),
        scratch_shapes=[pltpu.VMEM((6, K, 3 * C), jnp.bfloat16)],
        compiler_params=pltpu.CompilerParams(
            dimension_semantics=("arbitrary",), vmem_limit_bytes=100 * 2**20),
    )(xt, xt, xt, wt)
    return out.transpose(0, 2, 1).reshape(N, H, W, K)
```
